```python
import os as _os
_os.environ.setdefault("JAX_PLATFORMS", "cpu")
import jax
import jax.numpy as jnp

def _softmax(x, axis=-1):
    return jax.nn.softmax(x, axis=axis)
def _gelu(x):
    return jax.nn.gelu(x, approximate=True)
def _silu(x):
    return jax.nn.silu(x)
def _sigmoid(x):
    return jax.nn.sigmoid(x)
def _layernorm(x, axis=-1, eps=1e-5):
    m = jnp.mean(x, axis=axis, keepdims=True)
    v = jnp.var(x, axis=axis, keepdims=True)
    return (x - m) / jnp.sqrt(v + eps)
def _scatter_add(tgt, idx, src, axis=0):
    return tgt.at[idx].add(src)
def _segment_sum(src, seg, n):
    return jax.ops.segment_sum(src, seg, n)
class _Rng:
    def __init__(self, key):
        self._k = key
    def _next(self):
        self._k, sub = jax.random.split(self._k)
        return sub
    def normal(self, shape):
        return jax.random.normal(self._next(), shape, dtype=jnp.bfloat16)
    def randint(self, lo, hi, shape):
        return jax.random.randint(self._next(), shape, lo, hi, dtype=jnp.int32)
    def uniform(self, shape, lo=0.0, hi=1.0):
        return jax.random.uniform(self._next(), shape, jnp.bfloat16, lo, hi)
    def permutation(self, n):
        return jax.random.permutation(self._next(), n)


kernel_name = 'recurrent_scan__ssm_conv_s5__mixer_s_mlp__prompt'

def setup_inputs():
    _rng = _Rng(jax.random.key(int.from_bytes(__import__("os").urandom(4), "little")))
    _w = (lambda a: (lambda t: t.astype(jnp.bfloat16) if jnp.issubdtype(t.dtype, jnp.floating) else t)(jnp.asarray(a)))
    def _A_setup():
        B, S, D = 1, 2048, 640
        P = D
        Lambda_re = -0.5 * jnp.exp((lambda *s: _rng.normal(s) * 0.8)(P))
        Lambda_im = (lambda *s: _rng.normal(s) * 0.8)(P) * 1.0
        B_re = (lambda *s: _rng.normal(s) * 0.8)(P, D) * (D ** -0.5)
        B_im = (lambda *s: _rng.normal(s) * 0.8)(P, D) * (D ** -0.5)
        C_re = (lambda *s: _rng.normal(s) * 0.8)(D, P) * (P ** -0.5)
        C_im = (lambda *s: _rng.normal(s) * 0.8)(D, P) * (P ** -0.5)
        log_dt = (lambda *s: _rng.normal(s) * 0.8)(P) * 0.3 - 2.0
        Dskip = (lambda *s: _rng.normal(s) * 0.8)(D)
        return {
            "x": _w((lambda *s: _rng.normal(s) * 0.05)(B, S, D)),
            "Lambda_re": _w(Lambda_re),
            "Lambda_im": _w(Lambda_im),
            "B_re": _w(B_re),
            "B_im": _w(B_im),
            "C_re": _w(C_re),
            "C_im": _w(C_im),
            "log_dt": _w(log_dt),
            "Dskip": _w(Dskip),
        }
    _A_in = _A_setup()

    def _B_setup():
        B, S, D, F = 1, 2048, 640, 1536
        return {
            "x":  _w((lambda *s: _rng.normal(s) * 0.05)(B, S, D)),
            "w1": _w((lambda *s: _rng.normal(s) * 0.8)(D, D) * (D ** -0.5)),
            "w2": _w((lambda *s: _rng.normal(s) * 0.8)(D, D) * (D ** -0.5)),
            "w3": _w((lambda *s: _rng.normal(s) * 0.8)(D, F) * (D ** -0.5)),
            "w4": _w((lambda *s: _rng.normal(s) * 0.8)(F, D) * (F ** -0.5)),
        }
    _B_in = _B_setup()

    return {
        "A_x": _A_in["x"],
        "A_Lambda_re": _A_in["Lambda_re"],
        "A_Lambda_im": _A_in["Lambda_im"],
        "A_B_re": _A_in["B_re"],
        "A_B_im": _A_in["B_im"],
        "A_C_re": _A_in["C_re"],
        "A_C_im": _A_in["C_im"],
        "A_log_dt": _A_in["log_dt"],
        "A_Dskip": _A_in["Dskip"],
        "B_x": _B_in["x"],
        "B_w1": _B_in["w1"],
        "B_w2": _B_in["w2"],
        "B_w3": _B_in["w3"],
        "B_w4": _B_in["w4"],
    }

def reference(A_x, A_Lambda_re, A_Lambda_im, A_B_re, A_B_im, A_C_re, A_C_im, A_log_dt, A_Dskip, B_x, B_w1, B_w2, B_w3, B_w4):
    def _A_ref(x, Lambda_re, Lambda_im, B_re, B_im, C_re, C_im, log_dt, Dskip):
        Bsz, L, H = x.shape
        Lam = Lambda_re + 1j * Lambda_im
        Bmat = B_re + 1j * B_im
        Cmat = C_re + 1j * C_im
        dt = jnp.exp(log_dt)
        Lam_bar = jnp.exp(dt * Lam)
        B_bar = ((Lam_bar - 1.0) / Lam)[:, None] * Bmat
        Bu = jnp.einsum("bld,pd->blp", x + 0j, B_bar)
        h = jnp.zeros_like(Bu[:, 0, :])
        hs = []
        for t in range(L):
            h = Lam_bar[None, :] * h + Bu[:, t, :]
            hs.append(h)
        hseq = jnp.stack(hs, 1)
        y = 2.0 * jnp.einsum("blp,dp->bld", hseq, Cmat).real + x * Dskip[None, None, :]
        return y

    def _B_ref(x, w1, w2, w3, w4):
        B, S, D = x.shape
        h = _gelu(_layernorm(x, axis=-1) @ w1)
        c = D // 4
        g0 = jnp.pad(h[:, :, 0*c:1*c], ((0, 0), (1, 0), (0, 0)))[:, :S, :]
        g1 = jnp.pad(h[:, :, 1*c:2*c], ((0, 0), (0, 1), (0, 0)))[:, 1:, :]
        g2 = jnp.pad(h[:, :, 2*c:3*c], ((0, 0), (2, 0), (0, 0)))[:, :S, :]
        g3 = jnp.pad(h[:, :, 3*c:   ], ((0, 0), (0, 2), (0, 0)))[:, 2:, :]
        hs = jnp.concatenate([g0, g1, g2, g3], axis=-1) @ w2
        x1 = x + hs
        h2 = _gelu(_layernorm(x1, axis=-1) @ w3) @ w4
        return x1 + h2

    x = A_x
    xn = _layernorm(x, axis=-1)
    s = _A_ref(xn, A_Lambda_re, A_Lambda_im, A_B_re, A_B_im, A_C_re, A_C_im, A_log_dt, A_Dskip)
    g = _silu(_B_ref(xn, B_w1, B_w2, B_w3, B_w4))
    return x + s * g
```

```python
import jax
import jax.numpy as jnp
from jax import lax
import jax.experimental.pallas as pl
import jax.experimental.pallas.tpu as pltpu

L, D, F, P = 2048, 640, 1536, 640
T = 128
LEAD = 6
UM, UE = 2, 3
NB = L // T
TC = T // 8
NT = D // 128
NF = F // 128
XP = TC + 1
OP = 9
SG = 4
EPS = 1e-5
f32, bf16, u32 = jnp.float32, jnp.bfloat16, jnp.uint32


def _ln(x):
    m = jnp.mean(x, axis=-1, keepdims=True)
    xc = x - m
    v = jnp.mean(xc * xc, axis=-1, keepdims=True)
    return xc * lax.rsqrt(v + EPS)


def _gelu(x):
    c = 0.7978845608028654
    inner = x * (c + (c * 0.044715) * (x * x))
    hx = 0.5 * x
    return hx + hx * jnp.tanh(inner)


def _nn(a, b):
    return lax.dot_general(a, b, (((1,), (0,)), ((), ())), preferred_element_type=f32)


def _nt(a, b):
    return lax.dot_general(a, b, (((1,), (1,)), ((), ())), preferred_element_type=f32)


def _lt(a, j):
    return a[:, 128 * j:128 * (j + 1)]


def _sum(xs):
    acc = xs[0]
    for v in xs[1:]:
        acc = acc + v
    return acc


def kernel(x_hbm, lre_hbm, lim_hbm, bre_hbm, bim_hbm, cre_hbm, cim_hbm, ldt_hbm, dsk_hbm,
           w1_hbm, w2_hbm, w3_hbm, w4_hbm, out_hbm,
           x_v, lre_v, lim_v, ldt_v, dsk_v, bre_v, bim_v, cre_v, cim_v, w1_v, w2_v, w3_v, w4_v,
           xs_v, os_v, o_v, xn_v, g_v, s_v, psems, wsems, xsems, osems, fsem):
    def wcopies(w_hbm, w_v, n, k):
        return [pltpu.make_async_copy(w_hbm.at[:, pl.ds(128 * j, 128)], w_v.bitcast(bf16).at[j], wsems.at[k])
                for j in range(n)]

    def xcopy(r0, r1, k):
        return [pltpu.make_async_copy(x_hbm.at[pl.ds(r0, r1 - r0)], x_v.at[pl.ds(r0, r1 - r0)], xsems.at[k])]

    XA, XB = 256, LEAD * T
    groups = {
        "par": [pltpu.make_async_copy(s, d, psems.at[k]) for k, (s, d) in
                enumerate(((lre_hbm, lre_v), (lim_hbm, lim_v), (ldt_hbm, ldt_v), (dsk_hbm, dsk_v)))],
        "w1": wcopies(w1_hbm, w1_v, NT, 0),
        "B": wcopies(bre_hbm, bre_v, NT, 1) + wcopies(bim_hbm, bim_v, NT, 2),
        "C": wcopies(cre_hbm, cre_v, NT, 3) + wcopies(cim_hbm, cim_v, NT, 4),
        "w2": wcopies(w2_hbm, w2_v, NT, 5),
        "w3": wcopies(w3_hbm, w3_v, NF, 6),
        "w4": wcopies(w4_hbm, w4_v, NT, 7),
        "x0": xcopy(0, XA, 0), "x1": xcopy(XA, XB, 1), "xr": xcopy(XB, L, 2),
    }
    plan = {"t0": ["x0", "|", "w1", "|", "x1", "par"], "w1": ["B"], "x1": ["C"], "B": ["w2", "w3"],
            "i0": ["w4"], "i1": ["xr"]}

    def issue(point):
        for g in plan.get(point, ()):
            if g == "|":
                pl.semaphore_signal(fsem, 1)
                pl.semaphore_wait(fsem, 1)
            else:
                for c in groups[g]: c.start()

    def need(*names):
        for name in names:
            for c in groups[name]: c.wait()
        for name in names:
            issue(name)

    def rows(i):
        return pl.ds(i * T, T) if isinstance(i, int) else pl.ds(pl.multiple_of(i * T, T), T)

    def ocp(i, j):
        return pltpu.make_async_copy(o_v.at[i * NT + j], out_hbm.at[rows(i), pl.ds(128 * j, 128)], osems.at[i])

    def wtile(w_v, j, k=None):
        if k is None:
            return pltpu.bitcast(w_v[j], bf16)
        return pltpu.bitcast(w_v[j, pl.ds(64 * k, 64), :], bf16)

    def nn_full(a, w_v, j):
        return _nn(a, wtile(w_v, j))

    def nn_parts(parts, w_v, j):
        return _sum([_nn(p, wtile(w_v, j, k)) for k, p in enumerate(parts)])

    def nt_full(a, w_v, j):
        return _nt(a, pltpu.bitcast(jnp.concatenate([w_v[k, pl.ds(64 * j, 64), :] for k in range(NT)], axis=1), bf16))

    def nt_parts(parts, w_v, j):
        return _sum([_nt(p, wtile(w_v, k, j)) for k, p in enumerate(parts)])

    row8 = lax.broadcasted_iota(jnp.int32, (8, 128), 0)
    lane = lax.broadcasted_iota(jnp.int32, (T, 128), 1)
    prm = {}

    def params():
        lre = lre_v[...].astype(f32).reshape(1, P)
        lim = lim_v[...].astype(f32).reshape(1, P)
        dt = jnp.exp(ldt_v[...].astype(f32)).astype(bf16).astype(f32).reshape(1, P)
        prm["dsk"] = dsk_v[...].astype(f32).reshape(1, D)
        zr, zi = dt * lre, dt * lim
        r8 = lax.broadcasted_iota(jnp.int32, (8, P), 0)
        k = jnp.where(r8 == 0, 1.0, jnp.where(r8 == 1, float(TC), jnp.where(r8 == 2, 2.0 * TC, 4.0 * TC)))
        mag = jnp.exp(k * zr)
        pr, pi = mag * jnp.cos(k * zi), mag * jnp.sin(k * zi)
        ar, ai = pr[0:1], pi[0:1]
        den = lre * lre + lim * lim
        gr = ((ar - 1.0) * lre + ai * lim) / den
        gi = (ai * lre - (ar - 1.0) * lim) / den
        b8 = lambda v: jnp.broadcast_to(v, (8, P))
        prm["a"] = (b8(ar), b8(ai))
        prm["g"] = (b8(gr), b8(gi))
        prm["m"] = [(jnp.where(r8 >= sh, b8(pr[q:q + 1]), 0.0), jnp.where(r8 >= sh, b8(pi[q:q + 1]), 0.0))
                    for q, sh in ((1, 1), (2, 2), (3, 4))]

    NLN = TC // SG

    def xperm(i, j, t0, n):
        return jnp.concatenate([xs_v[i * NT + j, pl.ds(t, 8, stride=XP), :] for t in range(t0, t0 + n)], axis=0)

    def a01(i):
        for j in range(NT):
            xf = x_v[rows(i), pl.ds(128 * j, 128)].astype(f32)
            for c in range(8):
                xs_v[i * NT + j, pl.ds(XP * c, TC), :] = xf[TC * c:TC * (c + 1)]
        xn, l2 = [], []
        for q in range(NLN):
            x = jnp.concatenate([xperm(i, j, q * SG, SG) for j in range(NT)], axis=1)
            v = _ln(x)
            xn.append(v)
            l2.append(_ln(v))
        xn = jnp.concatenate(xn, axis=0)
        xn_v[i] = xn
        return xn, jnp.concatenate(l2, axis=0).astype(bf16)

    def a2(i, l2):
        for j in range(NT):
            g_v[i + 1, :, pl.ds(128 * j, 128)] = _gelu(nn_full(l2, w1_v, j))

    def a4(xn, carry):
        xb = xn.astype(bf16)
        hrs, his, new = [], [], []
        for j in range(NT):
            ar, ai = _lt(prm["a"][0], j), _lt(prm["a"][1], j)
            gr, gi = _lt(prm["g"][0], j), _lt(prm["g"][1], j)
            ur0, ui0 = nt_full(xb, bre_v, j), nt_full(xb, bim_v, j)
            vr, vi = [], []
            for t in range(TC):
                a, b = ur0[8 * t:8 * t + 8], ui0[8 * t:8 * t + 8]
                vr.append(a * gr - b * gi)
                vi.append(a * gi + b * gr)
            fr, fi = vr[0], vi[0]
            for t in range(1, TC):
                fr, fi = (fr * ar - fi * ai) + vr[t], (fr * ai + fi * ar) + vi[t]
            er = jnp.where(row8 >= 1, pltpu.roll(fr, 1, 0), carry[2 * j])
            ei = jnp.where(row8 >= 1, pltpu.roll(fi, 1, 0), carry[2 * j + 1])
            for sh, (mr, mi) in zip((1, 2, 4), prm["m"]):
                mr, mi = _lt(mr, j), _lt(mi, j)
                sr = pltpu.roll(er, sh, 0); si = pltpu.roll(ei, sh, 0)
                er, ei = er + (sr * mr - si * mi), ei + (sr * mi + si * mr)
            hr, hi = er, ei
            o_r, o_i = [], []
            for t in range(TC):
                hr, hi = (hr * ar - hi * ai) + vr[t], (hr * ai + hi * ar) + vi[t]
                o_r.append(hr); o_i.append(hi)
            new += [jnp.broadcast_to(hr[7:8, :], (8, 128)), jnp.broadcast_to(hi[7:8, :], (8, 128))]
            hrs.append(jnp.concatenate(o_r, 0).astype(bf16))
            his.append(jnp.concatenate(o_i, 0).astype(bf16))
        return hrs, his, tuple(new)

    def sdiag(xn):
        return [_lt(xn, j) * _lt(prm["dsk"], j) for j in range(NT)]

    def b6(i, hr, hi, xd):
        for j in range(NT):
            yc = nt_parts(hr, cre_v, j) - nt_parts(hi, cim_v, j)
            s_v[i, :, pl.ds(128 * j, 128)] = (yc + yc) + xd[j]

    def edge(i, j, t, down):
        ls = pl.ds(128 * j, 128)
        cur = g_v[i + 1, pl.ds(8 * t, 8), ls]
        other = g_v[i if down else i + 2, pl.ds(8 * t, 8), ls]
        if down:
            return pltpu.roll(jnp.where(row8 == 7, other, cur), 1, 0)
        return pltpu.roll(jnp.where(row8 == 0, other, cur), 7, 0)

    def shifted(i, j, sh):
        ls = pl.ds(128 * j, 128)
        if sh > 0:
            return jnp.concatenate([edge(i, j, TC - sh + k, True) for k in range(sh)] + [g_v[i + 1, pl.ds(0, T - 8 * sh), ls]], axis=0)
        sh = -sh
        return jnp.concatenate([g_v[i + 1, pl.ds(8 * sh, T - 8 * sh), ls]] + [edge(i, j, k, False) for k in range(sh)], axis=0)

    def b12(i):
        cols = [shifted(i, 0, 1),
                jnp.where(lane < 32, shifted(i, 1, 1), shifted(i, 1, -1)),
                jnp.where(lane < 64, shifted(i, 2, -1), shifted(i, 2, 2)),
                jnp.where(lane < 96, shifted(i, 3, 2), shifted(i, 3, -2)),
                shifted(i, 4, -2)]
        g = [c.astype(bf16) for c in cols]
        return [xn_v[i, :, pl.ds(128 * j, 128)] + nn_parts(g, w2_v, j) for j in range(NT)]

    def b3(x1):
        l3 = []
        for q in range(NLN):
            r = slice(8 * SG * q, 8 * SG * (q + 1))
            l3.append(_ln(jnp.concatenate([c[r] for c in x1], axis=1)))
        return jnp.concatenate(l3, axis=0).astype(bf16)

    def b4(l3):
        return [_gelu(nn_full(l3, w3_v, j)).astype(bf16) for j in range(NF)]

    def b5(i, m, x1):
        for j in range(NT):
            hb = 0.5 * (x1[j] + nn_parts(m, w4_v, j))
            gate = hb + hb * jnp.tanh(hb)
            o = s_v[i, :, pl.ds(128 * j, 128)] * gate
            k = i * NT + j
            for t in range(TC):
                os_v[k, pl.ds(OP * t, 8), :] = o[8 * t:8 * t + 8]
            for c in range(8):
                for q in range(TC // 8):
                    v = xs_v[k, pl.ds(XP * c + 8 * q, 8), :] + os_v[k, pl.ds(OP * 8 * q + c, 8, stride=OP), :]
                    o_v[k, pl.ds(TC * c + 8 * q, 8), :] = v
            ocp(i, j).start()

    issue("t0")
    g_v[0] = jnp.zeros((T, D), f32)
    g_v[NB + 1] = jnp.zeros((T, D), f32)
    G = XA // T
    need("x0")
    pre = {i: a01(i) for i in range(G)}
    need("w1")
    a2(0, pre[0][1])
    need("x1", "par")
    nl = G
    for i in range(1, LEAD):
        while nl < LEAD and nl <= i + 1:
            pre[nl] = a01(nl); nl += 1
        if i == LEAD - 2: params()
        a2(i, pre[i][1])
    need("B")
    carry = tuple(jnp.zeros((8, 128), f32) for _ in range(2 * NT))
    hh = {}
    for i in range(LEAD):
        hr, hi, carry = a4(pre[i][0], carry)
        hh[i] = (hr, hi)
        if i == 0: issue("i0")
        if i == 1: issue("i1")
        if i == LEAD - 2: need("C")
    for i in range(LEAD):
        b6(i, hh[i][0], hh[i][1], sdiag(pre[i][0]))
    need("w2", "w3", "w4", "xr")

    def main_one(i, carry):
        j = i + LEAD
        x1 = b12(i)
        xn, l2 = a01(j)
        a2(j, l2)
        l3 = b3(x1)
        m = b4(l3)
        hr, hi, carry = a4(xn, carry)
        b5(i, m, x1)
        b6(j, hr, hi, sdiag(xn))
        return carry

    def main_body(k, carry):
        for u in range(UM):
            carry = main_one(k * UM + u, carry)
        return carry
    assert (NB - LEAD) % UM == 0 and LEAD % UE == 0
    lax.fori_loop(0, (NB - LEAD) // UM, main_body, carry)

    def tail_body(k, c):
        i0 = NB - LEAD + k * UE
        x1 = [b12(i0 + u) for u in range(UE)]
        m = []
        for u in range(UE):
            m.append(b4(b3(x1[u])))
        for u in range(UE):
            b5(i0 + u, m[u], x1[u])
        return c
    lax.fori_loop(0, LEAD // UE, tail_body, 0)

    for i in range(NB):
        for j in range(NT):
            ocp(i, j).wait()


@jax.jit
def pallas_recurrent_scan__ssm_conv_s5__mixer_s_mlp__prompt_kernel(
        A_x, A_Lambda_re, A_Lambda_im, A_B_re, A_B_im, A_C_re, A_C_im, A_log_dt, A_Dskip,
        B_x, B_w1, B_w2, B_w3, B_w4):
    del B_x
    x = A_x.reshape(L, D)
    any_spec = pl.BlockSpec(memory_space=pl.ANY)
    V = pltpu.VMEM
    out = pl.pallas_call(
        kernel,
        out_shape=jax.ShapeDtypeStruct((L, D), f32),
        in_specs=[any_spec] * 13,
        out_specs=any_spec,
        scratch_shapes=[
            V((L, D), bf16), V((P,), bf16), V((P,), bf16), V((P,), bf16), V((D,), bf16),
            V((NT, P // 2, 128), u32), V((NT, P // 2, 128), u32), V((NT, D // 2, 128), u32), V((NT, D // 2, 128), u32),
            V((NT, D // 2, 128), u32), V((NT, D // 2, 128), u32), V((NF, D // 2, 128), u32), V((NT, F // 2, 128), u32),
            V((NB * NT, 8 * XP, 128), f32), V((NB * NT, TC * OP, 128), f32), V((NB * NT, T, 128), f32),
            V((NB, T, D), f32), V((NB + 2, T, D), f32), V((NB, T, D), f32),
            pltpu.SemaphoreType.DMA((4,)), pltpu.SemaphoreType.DMA((8,)), pltpu.SemaphoreType.DMA((3,)),
            pltpu.SemaphoreType.DMA((NB,)), pltpu.SemaphoreType.REGULAR,
        ],
        compiler_params=pltpu.CompilerParams(vmem_limit_bytes=100 * 1024 * 1024),
    )(x, A_Lambda_re, A_Lambda_im, A_B_re, A_B_im, A_C_re, A_C_im, A_log_dt, A_Dskip, B_w1, B_w2, B_w3, B_w4)
    return out.reshape(1, L, D)
```
